```python
import os as _os
_os.environ.setdefault("JAX_PLATFORMS", "cpu")
import jax
import jax.numpy as jnp

def _softmax(x, axis=-1):
    return jax.nn.softmax(x, axis=axis)
def _gelu(x):
    return jax.nn.gelu(x, approximate=True)
def _silu(x):
    return jax.nn.silu(x)
def _sigmoid(x):
    return jax.nn.sigmoid(x)
def _layernorm(x, axis=-1, eps=1e-5):
    m = jnp.mean(x, axis=axis, keepdims=True)
    v = jnp.var(x, axis=axis, keepdims=True)
    return (x - m) / jnp.sqrt(v + eps)
def _scatter_add(tgt, idx, src, axis=0):
    return tgt.at[idx].add(src)
def _segment_sum(src, seg, n):
    return jax.ops.segment_sum(src, seg, n)
class _Rng:
    def __init__(self, key):
        self._k = key
    def _next(self):
        self._k, sub = jax.random.split(self._k)
        return sub
    def normal(self, shape):
        return jax.random.normal(self._next(), shape, dtype=jnp.bfloat16)
    def randint(self, lo, hi, shape):
        return jax.random.randint(self._next(), shape, lo, hi, dtype=jnp.int32)
    def uniform(self, shape, lo=0.0, hi=1.0):
        return jax.random.uniform(self._next(), shape, jnp.bfloat16, lo, hi)
    def permutation(self, n):
        return jax.random.permutation(self._next(), n)


kernel_name = 'standalone__mha_softmax__sampling'

def setup_inputs():
    _rng = _Rng(jax.random.key(int.from_bytes(__import__("os").urandom(4), "little")))
    _w = (lambda a: (lambda t: t.astype(jnp.bfloat16) if jnp.issubdtype(t.dtype, jnp.floating) else t)(jnp.asarray(a)))
    B, H, Sq, Sk, D = 8, 32, 32, 2048, 128
    return {
        "q": _w((lambda *s: _rng.normal(s) * 0.4)(B, H, Sq, D)),
        "k": _w((lambda *s: _rng.normal(s) * 0.4)(B, H, Sk, D)),
        "v": _w((lambda *s: _rng.normal(s) * 0.05)(B, H, Sk, D)),
    }

def reference(q, k, v):
    scale = q.shape[-1] ** -0.5
    scores = jnp.einsum("bhqd,bhkd->bhqk", q, k) * scale
    p = _softmax(scores, axis=-1)
    return jnp.einsum("bhqk,bhkd->bhqd", p, v)
```

```python
import functools
import math

import jax
import jax.numpy as jnp
import numpy as np
from jax import lax
from jax.experimental import pallas as pl
from jax.experimental.pallas import tpu as pltpu

LANES = 128
ROWS = 128
HEADS = 8
CHUNKS = 4
AHEAD = 2
SLOTS = AHEAD + 1


def _mha_kernel(q_hbm, k_hbm, v_hbm, o_hbm,
                q_buf, k_buf, v_buf, o_buf, m_ref, l_ref, acc_ref,
                k_sem, v_sem, q_sem, o_sem):
    heads, groups, sk, d = k_hbm.shape
    sq = q_hbm.shape[2]
    keys = k_buf.shape[2]
    units_per_group = sk // keys
    units = groups * units_per_group
    c = (d ** -0.5) * math.log2(math.e)

    def fetch(unit, slot):
        j, u = unit // units_per_group, unit % units_per_group
        for r in range(0, keys, ROWS):
            row = pl.multiple_of(u * keys + r, ROWS)
            for g in range(heads):
                for prio, (src, dst, sem) in enumerate(
                        ((k_hbm, k_buf, k_sem), (v_hbm, v_buf, v_sem))):
                    pltpu.make_async_copy(
                        src.at[g, j, pl.ds(row, ROWS)],
                        dst.at[slot, g, pl.ds(r, ROWS)],
                        sem.at[slot],
                    ).start(priority=prio)

    def store_out(j0, n, sem):
        return pltpu.make_async_copy(
            o_buf.at[:, pl.ds(j0, n)], o_hbm.at[:, pl.ds(j0, n)], sem)

    q_copy = pltpu.make_async_copy(q_hbm, q_buf, q_sem.at[0])
    fetch(0, 0)
    q_copy.start()
    for unit in range(1, AHEAD):
        fetch(unit, unit)
    q_copy.wait()

    def step(unit, slot):
        j, u = unit // units_per_group, unit % units_per_group

        @pl.when(u == 0)
        def _():
            m_ref[...] = jnp.full(m_ref.shape, np.finfo(np.float32).min, jnp.float32)
            l_ref[...] = jnp.zeros(l_ref.shape, jnp.float32)
            acc_ref[...] = jnp.zeros(acc_ref.shape, jnp.float32)

        @pl.when(unit == units - 1)
        def _():
            store_out(0, groups - 1, o_sem.at[0]).start()

        pltpu.make_async_copy(k_buf.at[slot], k_buf.at[slot], k_sem.at[slot]).wait()
        pltpu.make_async_copy(v_buf.at[slot], v_buf.at[slot], v_sem.at[slot]).wait()

        @pl.when(unit + AHEAD < units)
        def _():
            nxt = slot + AHEAD
            fetch(unit + AHEAD, jnp.where(nxt >= SLOTS, nxt - SLOTS, nxt))

        s = jnp.concatenate(
            [lax.dot_general(q_buf[g, j], k_buf[slot, g], (((1,), (1,)), ((), ())),
                             preferred_element_type=jnp.float32)
             for g in range(heads)], axis=0)
        parts = [s[:, i:i + LANES] for i in range(0, keys, LANES)]
        m_old = m_ref[...]
        m_new = jnp.maximum(
            m_old, jnp.max(functools.reduce(jnp.maximum, parts), axis=-1, keepdims=True))
        alpha = jnp.exp2((m_old - m_new) * c)
        ps = [jnp.exp2((x - m_new) * c) for x in parts]
        p = jnp.concatenate(ps, axis=1).astype(v_buf.dtype)
        pv = jnp.concatenate(
            [jnp.dot(p[g * sq:(g + 1) * sq], v_buf[slot, g],
                     preferred_element_type=jnp.float32)
             for g in range(heads)], axis=0)
        m_ref[...] = m_new
        l_ref[...] = alpha * l_ref[...] + functools.reduce(jnp.add, ps)
        acc_ref[...] = alpha * acc_ref[...] + pv

        @pl.when(u == units_per_group - 1)
        def _():
            o = acc_ref[...] / jnp.sum(l_ref[...], axis=-1, keepdims=True)
            o = o.astype(o_buf.dtype)
            for g in range(heads):
                o_buf[g, j] = o[g * sq:(g + 1) * sq]

        return jnp.where(slot == SLOTS - 1, 0, slot + 1)

    lax.fori_loop(0, units, step, jnp.int32(0))
    last = store_out(groups - 1, 1, o_sem.at[1])
    last.start()
    store_out(0, groups - 1, o_sem.at[0]).wait()
    last.wait()


@jax.jit
def pallas_standalone__mha_softmax__sampling_kernel(
    q: jax.Array,
    k: jax.Array,
    v: jax.Array,
):
    b, h, sq, d = q.shape
    sk = k.shape[2]
    keys = CHUNKS * ROWS
    assert d == LANES and (b * h) % HEADS == 0 and sk % keys == 0
    groups = (b * h) // HEADS
    hbm = pl.BlockSpec(memory_space=pl.ANY)
    out = pl.pallas_call(
        _mha_kernel,
        in_specs=[hbm, hbm, hbm],
        out_specs=hbm,
        out_shape=jax.ShapeDtypeStruct((HEADS, groups, sq, d), q.dtype),
        scratch_shapes=[
            pltpu.VMEM((HEADS, groups, sq, d), q.dtype),
            pltpu.VMEM((SLOTS, HEADS, keys, d), k.dtype),
            pltpu.VMEM((SLOTS, HEADS, keys, d), v.dtype),
            pltpu.VMEM((HEADS, groups, sq, d), q.dtype),
            pltpu.VMEM((HEADS * sq, LANES), jnp.float32),
            pltpu.VMEM((HEADS * sq, LANES), jnp.float32),
            pltpu.VMEM((HEADS * sq, d), jnp.float32),
            pltpu.SemaphoreType.DMA((SLOTS,)),
            pltpu.SemaphoreType.DMA((SLOTS,)),
            pltpu.SemaphoreType.DMA((1,)),
            pltpu.SemaphoreType.DMA((2,)),
        ],
        compiler_params=pltpu.CompilerParams(vmem_limit_bytes=48 * 2**20),
    )(
        q.reshape(HEADS, groups, sq, d),
        k.reshape(HEADS, groups, sk, d),
        v.reshape(HEADS, groups, sk, d),
    )
    return out.reshape(b, h, sq, d)
```

```python
import functools
import math

import jax
import jax.numpy as jnp
import numpy as np
from jax import lax
from jax.experimental import pallas as pl
from jax.experimental.pallas import tpu as pltpu

LANES = 128
ROWS = 128
HEADS = 8
CHUNKS = 4
AHEAD = 4
SLOTS = AHEAD + 1
OUT_PIECE = 6


def _mha_kernel(q_hbm, k_hbm, v_hbm, o_hbm,
                q_buf, kv_buf, o_buf, m_ref, l_ref, acc_ref, kv_sem, qo_sem):
    heads, groups, sk, d = k_hbm.shape
    sq = q_hbm.shape[2]
    keys = kv_buf.shape[3]
    units_per_group = sk // keys
    units = groups * units_per_group
    ahead = kv_buf.shape[0] - 1
    c = (d ** -0.5) * math.log2(math.e)

    def q_copy(j):
        return pltpu.make_async_copy(q_hbm.at[:, j], q_buf.at[:, j], qo_sem.at[0])

    def fetch(unit, slot):
        j, u = unit // units_per_group, unit % units_per_group
        for r in range(0, keys, ROWS):
            row = u * keys + r
            if not isinstance(row, int):
                row = pl.multiple_of(row, ROWS)
            for g in range(heads):
                for t, src in enumerate((k_hbm, v_hbm)):
                    pltpu.make_async_copy(
                        src.at[g, j, pl.ds(row, ROWS)],
                        kv_buf.at[slot, t, g, pl.ds(r, ROWS)],
                        kv_sem.at[slot],
                    ).start(priority=t)

    def store(j0, j1):
        for j in range(j0, j1, OUT_PIECE):
            for g in range(heads):
                piece = (g, pl.ds(j, min(OUT_PIECE, j1 - j)))
                pltpu.make_async_copy(
                    o_buf.at[piece], o_hbm.at[piece], qo_sem.at[0]
                ).start(priority=g % 2)

    q_copy(0).start()
    for unit in range(ahead):
        fetch(unit, unit)

    def step(unit, slot):
        j, u = unit // units_per_group, unit % units_per_group

        @pl.when(u == 0)
        def _():
            m_ref[...] = jnp.full(m_ref.shape, np.finfo(np.float32).min, jnp.float32)
            l_ref[...] = jnp.zeros(l_ref.shape, jnp.float32)
            acc_ref[...] = jnp.zeros(acc_ref.shape, jnp.float32)
            q_copy(j).wait()

        @pl.when(unit == units - 1)
        def _():
            store(0, groups - 1)

        pltpu.make_async_copy(kv_buf.at[slot], kv_buf.at[slot], kv_sem.at[slot]).wait()

        @pl.when(unit + ahead < units)
        def _():
            @pl.when(u == units_per_group - ahead)
            def _():
                q_copy(j + 1).start()

            fetch(unit + ahead, jnp.where(slot == 0, ahead, slot - 1))

        s = jnp.concatenate(
            [lax.dot_general(q_buf[g, j], kv_buf[slot, 0, g], (((1,), (1,)), ((), ())),
                             preferred_element_type=jnp.float32)
             for g in range(heads)], axis=0)
        parts = [s[:, i:i + LANES] for i in range(0, keys, LANES)]
        m_old = m_ref[...]
        m_new = jnp.maximum(
            m_old, jnp.max(functools.reduce(jnp.maximum, parts), axis=-1, keepdims=True))
        alpha = jnp.exp2((m_old - m_new) * c)
        ps = [jnp.exp2((x - m_new) * c) for x in parts]
        p = jnp.concatenate(ps, axis=1).astype(kv_buf.dtype)
        pv = jnp.concatenate(
            [jnp.dot(p[g * sq:(g + 1) * sq], kv_buf[slot, 1, g],
                     preferred_element_type=jnp.float32)
             for g in range(heads)], axis=0)
        m_ref[...] = m_new
        l_ref[...] = alpha * l_ref[...] + functools.reduce(jnp.add, ps)
        acc_ref[...] = alpha * acc_ref[...] + pv

        @pl.when(u == units_per_group - 1)
        def _():
            o = acc_ref[...] / jnp.sum(l_ref[...], axis=-1, keepdims=True)
            o = o.astype(o_buf.dtype)
            for g in range(heads):
                o_buf[g, j] = o[g * sq:(g + 1) * sq]

        return jnp.where(slot == ahead, 0, slot + 1)

    lax.fori_loop(0, units, step, jnp.int32(0))
    store(groups - 1, groups)
    pltpu.make_async_copy(o_buf, o_hbm, qo_sem.at[0]).wait()


@jax.jit
def pallas_standalone__mha_softmax__sampling_kernel(
    q: jax.Array,
    k: jax.Array,
    v: jax.Array,
):
    b, h, sq, d = q.shape
    sk = k.shape[2]
    keys = CHUNKS * ROWS
    assert d == LANES and (b * h) % HEADS == 0 and sk % keys == 0
    assert AHEAD <= sk // keys
    groups = (b * h) // HEADS
    hbm = pl.BlockSpec(memory_space=pl.ANY)
    out = pl.pallas_call(
        _mha_kernel,
        in_specs=[hbm, hbm, hbm],
        out_specs=hbm,
        out_shape=jax.ShapeDtypeStruct((HEADS, groups, sq, d), q.dtype),
        scratch_shapes=[
            pltpu.VMEM((HEADS, groups, sq, d), q.dtype),
            pltpu.VMEM((SLOTS, 2, HEADS, keys, d), k.dtype),
            pltpu.VMEM((HEADS, groups, sq, d), q.dtype),
            pltpu.VMEM((HEADS * sq, LANES), jnp.float32),
            pltpu.VMEM((HEADS * sq, LANES), jnp.float32),
            pltpu.VMEM((HEADS * sq, d), jnp.float32),
            pltpu.SemaphoreType.DMA((SLOTS,)),
            pltpu.SemaphoreType.DMA((1,)),
        ],
        compiler_params=pltpu.CompilerParams(vmem_limit_bytes=48 * 2**20),
    )(
        q.reshape(HEADS, groups, sq, d),
        k.reshape(HEADS, groups, sk, d),
        v.reshape(HEADS, groups, sk, d),
    )
    return out.reshape(b, h, sq, d)
```
